```python
import jax
import jax.numpy as jnp

def _softmax(x, axis=-1):
    return jax.nn.softmax(x, axis=axis)
def _gelu(x):
    return jax.nn.gelu(x, approximate=True)
def _silu(x):
    return jax.nn.silu(x)
def _sigmoid(x):
    return jax.nn.sigmoid(x)
def _layernorm(x, axis=-1, eps=1e-5):
    m = jnp.mean(x, axis=axis, keepdims=True)
    v = jnp.var(x, axis=axis, keepdims=True)
    return (x - m) / jnp.sqrt(v + eps)
def _scatter_add(tgt, idx, src, axis=0):
    return tgt.at[idx].add(src)
def _segment_sum(src, seg, n):
    return jax.ops.segment_sum(src, seg, n)
class _Rng:
    def __init__(self, key):
        self._k = key
    def _next(self):
        self._k, sub = jax.random.split(self._k)
        return sub
    def normal(self, shape):
        return jax.random.normal(self._next(), shape, dtype=jnp.bfloat16)
    def randint(self, lo, hi, shape):
        return jax.random.randint(self._next(), shape, lo, hi, dtype=jnp.int32)
    def uniform(self, shape, lo=0.0, hi=1.0):
        return jax.random.uniform(self._next(), shape, jnp.bfloat16, lo, hi)
    def permutation(self, n):
        return jax.random.permutation(self._next(), n)


kernel_name = 'recurrent_scan__sliding_block_cached__dense_activation_gelu__decode'

def setup_inputs():
    _rng = _Rng(jax.random.key(int.from_bytes(__import__("os").urandom(4), "little")))
    _w = (lambda a: (lambda t: t.astype(jnp.bfloat16) if jnp.issubdtype(t.dtype, jnp.floating) else t)(jnp.asarray(a)))
    def _A_setup():
        B, Sq, D = 2, 1, 576
        Hq, Hkv, Sk, Dh = 32, 16, 32768, 128
        assert Hq % Hkv == 0, (Hq, Hkv)
        return {
            "x": _w((lambda *s: _rng.normal(s) * 0.05)(B, Sq, D)),
            "k_cache": _w((lambda *s: _rng.normal(s) * 0.05)(B, Hkv, Sk, Dh)),
            "v_cache": _w((lambda *s: _rng.normal(s) * 0.05)(B, Hkv, Sk, Dh)),
            "wq": _w((lambda *s: _rng.normal(s) * 0.05)(D, Hq * Dh) * (D ** -0.5)),
            "wo": _w((lambda *s: _rng.normal(s) * 0.05)(Hq * Dh, D) * ((Hq * Dh) ** -0.5)),
        }
    _A_in = _A_setup()

    def _B_setup():
        B, S, D, F = 2, 1, 576, 4608
        return {
            "x": _w((lambda *s: _rng.normal(s) * 0.05)(B, S, D)),
            "w1": _w((lambda *s: _rng.normal(s) * 0.05)(D, F) * (D ** -0.5)),
            "b1": _w((lambda *s: _rng.normal(s) * 0.05)(F) * 0.01),
            "w2": _w((lambda *s: _rng.normal(s) * 0.05)(F, D) * (F ** -0.5)),
            "b2": _w((lambda *s: _rng.normal(s) * 0.05)(D) * 0.01),
        }
    _B_in = _B_setup()

    return {
        "A_x": _A_in["x"],
        "A_k_cache": _A_in["k_cache"],
        "A_v_cache": _A_in["v_cache"],
        "A_wq": _A_in["wq"],
        "A_wo": _A_in["wo"],
        "B_x": _B_in["x"],
        "B_w1": _B_in["w1"],
        "B_b1": _B_in["b1"],
        "B_w2": _B_in["w2"],
        "B_b2": _B_in["b2"],
    }

def reference(A_x, A_k_cache, A_v_cache, A_wq, A_wo, B_x, B_w1, B_b1, B_w2, B_b2):
    def _A_ref(x, k_cache, v_cache, wq, wo):
        B, Sq, D = x.shape
        Hq, Dh = 32, 128
        Hkv, Sk = k_cache.shape[1], k_cache.shape[2]
        W = min(4096, max(256, Sk // 4))
        rep = Hq // Hkv
        q = (lambda x, *d: x.transpose(*d))((x @ wq).reshape(B, Sq, Hq, Dh), 0, 2, 1, 3)
        k = jnp.repeat(k_cache[:, :, Sk - W:, :], rep, axis=1)
        v = jnp.repeat(v_cache[:, :, Sk - W:, :], rep, axis=1)
        scores = jnp.einsum("bhqd,bhkd->bhqk", q, k) * (Dh ** -0.5)
        p = _softmax(scores, axis=-1)
        o = jnp.einsum("bhqk,bhkd->bhqd", p, v)
        return (lambda x, *d: x.transpose(*d))(o, 0, 2, 1, 3).reshape(B, Sq, Hq * Dh) @ wo

    def _B_ref(x, w1, b1, w2, b2):
        h = jnp.einsum("bsd,df->bsf", x, w1) + b1
        h = _gelu(h)
        return jnp.einsum("bsf,fd->bsd", h, w2) + b2

    x = A_x
    xn = _layernorm(x, axis=-1)
    s = _A_ref(xn, A_k_cache, A_v_cache, A_wq, A_wo)
    g = _silu(_B_ref(xn, B_w1, B_b1, B_w2, B_b2))
    return x + s * g
```

```python
import functools

import jax
import jax.numpy as jnp
from jax import lax
import jax.experimental.pallas as pl
import jax.experimental.pallas.tpu as pltpu

_NT = (((1,), (1,)), ((), ()))
_HQ = 32
_DH = 128
_ROWS = 8


def _kernel(x_hbm, k_hbm, v_hbm, wq_hbm, wot_hbm, w1_hbm, b1_hbm, w2t_hbm, b2_hbm,
            out_ref,
            x_v, b1_v, b2_v, wq_v, w1_v, w2t_v, wot_v, kbuf, vbuf, q_scr, o_scr,
            sem_small, sem_w, sem_k, sem_v, sem_wo,
            *, n_batch, n_kv, window, seq, d_model, n_wo_chunks):
    rep = _HQ // n_kv
    assert rep == 2 and n_batch == 2
    wo_cw = (_HQ * _DH) // n_wo_chunks

    def x_copy():
        return pltpu.make_async_copy(x_hbm, x_v, sem_small.at[0])

    def b1_copy():
        return pltpu.make_async_copy(b1_hbm, b1_v, sem_small.at[1])

    def b2_copy():
        return pltpu.make_async_copy(b2_hbm, b2_v, sem_small.at[2])

    def wq_copy():
        return pltpu.make_async_copy(wq_hbm, wq_v, sem_w.at[0])

    def w1_copy():
        return pltpu.make_async_copy(w1_hbm, w1_v, sem_w.at[1])

    def w2_copy():
        return pltpu.make_async_copy(w2t_hbm, w2t_v, sem_w.at[2])

    def k_copy(h):
        return pltpu.make_async_copy(
            k_hbm.at[:, h, pl.ds(seq - window, window), :], kbuf.at[h], sem_k.at[h])

    def v_copy(h):
        return pltpu.make_async_copy(
            v_hbm.at[:, h, pl.ds(seq - window, window), :], vbuf.at[h], sem_v.at[h])

    def wo_copy(c):
        cols = pl.ds(c * wo_cw, wo_cw)
        return pltpu.make_async_copy(wot_hbm.at[:, cols], wot_v.at[:, cols], sem_wo.at[c])

    x_copy().start()
    wq_copy().start()
    b1_copy().start()
    b2_copy().start()
    w1_copy().start()
    w2_copy().start()

    def issue(h, carry):
        k_copy(h).start()
        v_copy(h).start()
        return carry

    lax.fori_loop(0, n_kv, issue, 0)
    for c in range(n_wo_chunks):
        wo_copy(c).start()

    row = lax.broadcasted_iota(jnp.int32, (_ROWS, _DH), 0)

    x_copy().wait()
    x = x_v[...].astype(jnp.float32)
    mu = jnp.mean(x, axis=-1, keepdims=True)
    xc = x - mu
    var = jnp.mean(xc * xc, axis=-1, keepdims=True)
    xn = xc / jnp.sqrt(var + 1e-5)
    xn8 = jnp.concatenate([xn] * (_ROWS // n_batch), axis=0).astype(jnp.bfloat16)

    wq_copy().wait()
    q_scr[...] = jnp.dot(xn8, wq_v[...], preferred_element_type=jnp.float32)

    b1_copy().wait()
    b2_copy().wait()
    w1_copy().wait()
    hid = jnp.dot(xn8, w1_v[...], preferred_element_type=jnp.float32)
    hid = hid + b1_v[...].astype(jnp.float32).reshape(1, -1)
    hid = jax.nn.gelu(hid, approximate=True).astype(jnp.bfloat16)
    w2_copy().wait()
    y = lax.dot_general(hid, w2t_v[...], _NT, preferred_element_type=jnp.float32)
    y = y + b2_v[...].astype(jnp.float32).reshape(1, -1)
    gate = y * jax.nn.sigmoid(y)

    scale = _DH ** -0.5
    srow = lax.broadcasted_iota(jnp.int32, (_ROWS, window), 0)

    def attend(h, carry):
        c0 = pl.multiple_of(h * (rep * _DH), rep * _DH)
        c1 = pl.multiple_of(h * (rep * _DH) + _DH, _DH)
        qh = jnp.where((row & 2) == 0, q_scr[:, pl.ds(c0, _DH)], q_scr[:, pl.ds(c1, _DH)])
        qh = qh.astype(jnp.bfloat16)
        k_copy(h).wait()
        s0 = lax.dot_general(qh, kbuf[h, 0], _NT, preferred_element_type=jnp.float32)
        s1 = lax.dot_general(qh, kbuf[h, 1], _NT, preferred_element_type=jnp.float32)
        s = jnp.where((srow & 1) == 0, s0, s1) * scale
        m = jnp.max(s, axis=-1, keepdims=True)
        p = jnp.exp(s - m)
        l = jnp.sum(p, axis=-1, keepdims=True)
        pb = p.astype(jnp.bfloat16)
        v_copy(h).wait()
        o0 = jnp.dot(pb, vbuf[h, 0], preferred_element_type=jnp.float32)
        o1 = jnp.dot(pb, vbuf[h, 1], preferred_element_type=jnp.float32)
        o = jnp.where((row & 1) == 0, o0, o1) / l
        o_scr[:, pl.ds(c0, _DH)] = o
        o_scr[:, pl.ds(c1, _DH)] = pltpu.roll(o, _ROWS - 2, 0)
        return carry

    lax.fori_loop(0, n_kv, attend, 0)

    acc = jnp.zeros((_ROWS, d_model), jnp.float32)
    for c in range(n_wo_chunks):
        wo_copy(c).wait()
        oc = o_scr[:, c * wo_cw:(c + 1) * wo_cw].astype(jnp.bfloat16)
        acc = acc + lax.dot_general(oc, wot_v[:, c * wo_cw:(c + 1) * wo_cw], _NT,
                                    preferred_element_type=jnp.float32)
    res = x + acc[0:n_batch] * gate[0:n_batch]
    out_ref[...] = res.astype(out_ref.dtype)


@jax.jit
def pallas_recurrent_scan__sliding_block_cached__dense_activation_gelu__decode_kernel(
    A_x: jax.Array,
    A_k_cache: jax.Array,
    A_v_cache: jax.Array,
    A_wq: jax.Array,
    A_wo: jax.Array,
    B_x: jax.Array,
    B_w1: jax.Array,
    B_b1: jax.Array,
    B_w2: jax.Array,
    B_b2: jax.Array,
):
    del B_x
    n_batch, sq, d_model = A_x.shape
    _, n_kv, seq, dh = A_k_cache.shape
    assert sq == 1 and dh == _DH
    window = min(4096, max(256, seq // 4))
    d_ff = B_w1.shape[1]
    n_wo_chunks = 8
    bf16 = jnp.bfloat16

    hbm = pl.BlockSpec(memory_space=pl.ANY)
    out = pl.pallas_call(
        functools.partial(_kernel, n_batch=n_batch, n_kv=n_kv, window=window, seq=seq,
                          d_model=d_model, n_wo_chunks=n_wo_chunks),
        out_shape=jax.ShapeDtypeStruct((n_batch, d_model), A_x.dtype),
        in_specs=[hbm] * 9,
        out_specs=pl.BlockSpec(memory_space=pltpu.VMEM),
        scratch_shapes=[
            pltpu.VMEM((n_batch, d_model), bf16),
            pltpu.VMEM((d_ff,), bf16),
            pltpu.VMEM((d_model,), bf16),
            pltpu.VMEM((d_model, _HQ * _DH), bf16),
            pltpu.VMEM((d_model, d_ff), bf16),
            pltpu.VMEM((d_model, d_ff), bf16),
            pltpu.VMEM((d_model, _HQ * _DH), bf16),
            pltpu.VMEM((n_kv, n_batch, window, _DH), bf16),
            pltpu.VMEM((n_kv, n_batch, window, _DH), bf16),
            pltpu.VMEM((_ROWS, _HQ * _DH), jnp.float32),
            pltpu.VMEM((_ROWS, _HQ * _DH), jnp.float32),
            pltpu.SemaphoreType.DMA((3,)),
            pltpu.SemaphoreType.DMA((3,)),
            pltpu.SemaphoreType.DMA((n_kv,)),
            pltpu.SemaphoreType.DMA((n_kv,)),
            pltpu.SemaphoreType.DMA((n_wo_chunks,)),
        ],
        compiler_params=pltpu.CompilerParams(vmem_limit_bytes=112 * 1024 * 1024),
    )(A_x.reshape(n_batch, d_model), A_k_cache, A_v_cache, A_wq, A_wo.T,
      B_w1, B_b1, B_w2.T, B_b2)
    return out.reshape(n_batch, sq, d_model)
```

```python
import functools

import jax
import jax.numpy as jnp
from jax import lax
import jax.experimental.pallas as pl
import jax.experimental.pallas.tpu as pltpu

_NT = (((1,), (1,)), ((), ()))
_HQ = 32
_DH = 128
_ROWS = 8
_EPS = 1e-5


def _kernel(x_hbm, k_hbm, v_hbm, wq_hbm, wot_hbm, w1_hbm, b1_hbm, w2t_hbm, b2_hbm,
            out_ref,
            x_v, b1_v, b2_v, wq_v, w1_v, w2t_v, wot_v, kbuf, vbuf, q_scr, o_scr,
            sem_small, sem_w, sem_k, sem_v, sem_wo,
            *, n_batch, n_kv, window, seq, wo_pieces):
    rep = _HQ // n_kv
    assert rep == 2 and n_batch == 2

    def x_copy():
        return pltpu.make_async_copy(x_hbm, x_v, sem_small.at[0])

    def b1_copy():
        return pltpu.make_async_copy(b1_hbm, b1_v, sem_small.at[1])

    def b2_copy():
        return pltpu.make_async_copy(b2_hbm, b2_v, sem_small.at[2])

    def wq_copy():
        return pltpu.make_async_copy(wq_hbm, wq_v, sem_w.at[0])

    def w1_copy():
        return pltpu.make_async_copy(w1_hbm, w1_v, sem_w.at[1])

    def w2_copy():
        return pltpu.make_async_copy(w2t_hbm, w2t_v, sem_w.at[2])

    def k_copy(h):
        return pltpu.make_async_copy(
            k_hbm.at[:, h, pl.ds(seq - window, window), :], kbuf.at[h], sem_k.at[h])

    def v_copy(h):
        return pltpu.make_async_copy(
            v_hbm.at[:, h, pl.ds(seq - window, window), :], vbuf.at[h], sem_v.at[h])

    def wo_copy(c):
        r0, nr, c0, nc = wo_pieces[c]
        idx = (pl.ds(r0, nr), pl.ds(c0, nc))
        return pltpu.make_async_copy(wot_hbm.at[idx], wot_v.at[idx], sem_wo.at[c])

    wq_copy().start()
    x_copy().start()
    b1_copy().start()
    b2_copy().start()
    w1_copy().start()
    w2_copy().start()

    def issue(h, carry):
        k_copy(h).start()
        v_copy(h).start()
        return carry

    lax.fori_loop(0, n_kv, issue, 0)
    for c in range(len(wo_pieces)):
        wo_copy(c).start()

    x_copy().wait()
    x = x_v[...].astype(jnp.float32)
    x8 = jnp.concatenate([x] * (_ROWS // n_batch), axis=0)
    mu = jnp.mean(x8, axis=-1, keepdims=True)
    xc = x8 - mu
    var = jnp.mean(xc * xc, axis=-1, keepdims=True)
    xn8 = (xc / jnp.sqrt(var + _EPS)).astype(jnp.bfloat16)

    wq_copy().wait()
    q_scr[...] = jnp.dot(xn8, wq_v[...], preferred_element_type=jnp.float32)

    b1_copy().wait()
    b2_copy().wait()
    w1_copy().wait()
    hid = jnp.dot(xn8, w1_v[...], preferred_element_type=jnp.float32)
    hid = hid + b1_v[...].astype(jnp.float32).reshape(1, -1)
    hid = jax.nn.gelu(hid, approximate=True).astype(jnp.bfloat16)
    w2_copy().wait()
    y = lax.dot_general(hid, w2t_v[...], _NT, preferred_element_type=jnp.float32)
    y = y + b2_v[...].astype(jnp.float32).reshape(1, -1)
    gate = y * jax.nn.sigmoid(y)

    scale = _DH ** -0.5
    row = lax.broadcasted_iota(jnp.int32, (_ROWS, _DH), 0)
    srow = lax.broadcasted_iota(jnp.int32, (_ROWS, window), 0)

    def attend(h, carry):
        c0 = pl.multiple_of(h * (rep * _DH), rep * _DH)
        c1 = pl.multiple_of(h * (rep * _DH) + _DH, _DH)
        qh = jnp.where((row & 2) == 0, q_scr[:, pl.ds(c0, _DH)], q_scr[:, pl.ds(c1, _DH)])
        qh = qh.astype(jnp.bfloat16)
        k_copy(h).wait()
        s0 = lax.dot_general(qh, kbuf[h, 0], _NT, preferred_element_type=jnp.float32)
        s1 = lax.dot_general(qh, kbuf[h, 1], _NT, preferred_element_type=jnp.float32)
        s = jnp.where((srow & 1) == 0, s0, s1) * scale
        m = jnp.max(s, axis=-1, keepdims=True)
        p = jnp.exp(s - m)
        l = jnp.sum(p, axis=-1, keepdims=True)
        pb = p.astype(jnp.bfloat16)
        v_copy(h).wait()
        o0 = jnp.dot(pb, vbuf[h, 0], preferred_element_type=jnp.float32)
        o1 = jnp.dot(pb, vbuf[h, 1], preferred_element_type=jnp.float32)
        o = jnp.where((row & 1) == 0, o0, o1) / l
        o_scr[:, pl.ds(c0, _DH)] = o
        o_scr[:, pl.ds(c1, _DH)] = pltpu.roll(o, _ROWS - 2, 0)
        return carry

    lax.fori_loop(0, n_kv, attend, 0)

    partial = {}
    for c, (r0, nr, c0, nc) in enumerate(wo_pieces):
        oc = o_scr[:, c0:c0 + nc].astype(jnp.bfloat16)
        closes_group = c0 + nc == _HQ * _DH
        if closes_group:
            gs = gate[:, r0:r0 + nr]
            base = x8[:, r0:r0 + nr]
            if r0 in partial:
                base = base + partial[r0] * gs
        wo_copy(c).wait()
        part = lax.dot_general(oc, wot_v[r0:r0 + nr, c0:c0 + nc], _NT,
                               preferred_element_type=jnp.float32)
        if closes_group:
            res = base + part * gs
            out_ref[:, r0:r0 + nr] = res[0:n_batch].astype(out_ref.dtype)
        else:
            partial[r0] = part if r0 not in partial else partial[r0] + part


def _wo_pieces(d_model, k_total):
    pieces = []
    r = 0
    while d_model - r >= 128:
        pieces.append((r, 128, 0, k_total))
        r += 128
    if r < d_model:
        half = k_total // 2
        pieces.append((r, d_model - r, 0, half))
        pieces.append((r, d_model - r, half, k_total - half))
    return tuple(pieces)


@jax.jit
def pallas_recurrent_scan__sliding_block_cached__dense_activation_gelu__decode_kernel(
    A_x: jax.Array,
    A_k_cache: jax.Array,
    A_v_cache: jax.Array,
    A_wq: jax.Array,
    A_wo: jax.Array,
    B_x: jax.Array,
    B_w1: jax.Array,
    B_b1: jax.Array,
    B_w2: jax.Array,
    B_b2: jax.Array,
):
    del B_x
    n_batch, sq, d_model = A_x.shape
    _, n_kv, seq, dh = A_k_cache.shape
    assert sq == 1 and dh == _DH
    window = min(4096, max(256, seq // 4))
    d_ff = B_w1.shape[1]
    wo_pieces = _wo_pieces(d_model, _HQ * _DH)
    bf16 = jnp.bfloat16

    hbm = pl.BlockSpec(memory_space=pl.ANY)
    out = pl.pallas_call(
        functools.partial(_kernel, n_batch=n_batch, n_kv=n_kv, window=window, seq=seq,
                          wo_pieces=wo_pieces),
        out_shape=jax.ShapeDtypeStruct((n_batch, d_model), A_x.dtype),
        in_specs=[hbm] * 9,
        out_specs=pl.BlockSpec(memory_space=pltpu.VMEM),
        scratch_shapes=[
            pltpu.VMEM((n_batch, d_model), bf16),
            pltpu.VMEM((d_ff,), bf16),
            pltpu.VMEM((d_model,), bf16),
            pltpu.VMEM((d_model, _HQ * _DH), bf16),
            pltpu.VMEM((d_model, d_ff), bf16),
            pltpu.VMEM((d_model, d_ff), bf16),
            pltpu.VMEM((d_model, _HQ * _DH), bf16),
            pltpu.VMEM((n_kv, n_batch, window, _DH), bf16),
            pltpu.VMEM((n_kv, n_batch, window, _DH), bf16),
            pltpu.VMEM((_ROWS, _HQ * _DH), jnp.float32),
            pltpu.VMEM((_ROWS, _HQ * _DH), jnp.float32),
            pltpu.SemaphoreType.DMA((3,)),
            pltpu.SemaphoreType.DMA((3,)),
            pltpu.SemaphoreType.DMA((n_kv,)),
            pltpu.SemaphoreType.DMA((n_kv,)),
            pltpu.SemaphoreType.DMA((len(wo_pieces),)),
        ],
        compiler_params=pltpu.CompilerParams(
            vmem_limit_bytes=112 * 1024 * 1024,
            disable_semaphore_checks=True,
            disable_bounds_checks=True,
        ),
    )(A_x.reshape(n_batch, d_model), A_k_cache, A_v_cache, A_wq, A_wo.T,
      B_w1, B_b1, B_w2.T, B_b2)
    return out.reshape(n_batch, sq, d_model)
```

```python
import functools

import jax
import jax.numpy as jnp
from jax import lax
import jax.experimental.pallas as pl
import jax.experimental.pallas.tpu as pltpu

_NT = (((1,), (1,)), ((), ()))
_HQ = 32
_DH = 128
_ROWS = 8
_EPS = 1e-5


def _kernel(x_hbm, k_hbm, v_hbm, wq_hbm, wot_hbm, w1_hbm, b1_hbm, w2t_hbm, b2_hbm,
            out_ref,
            x_v, b1_v, b2_v, wq_v, w1_v, w2t_v, wot_v, kbuf, vbuf, q_scr, o_scr,
            sem_small, sem_w, sem_k, sem_v, sem_wo,
            *, n_batch, n_kv, window, seq, wo_pieces):
    rep = _HQ // n_kv
    assert rep == 2 and n_batch == 2

    def x_copy():
        return pltpu.make_async_copy(x_hbm, x_v, sem_small.at[0])

    def b1_copy():
        return pltpu.make_async_copy(b1_hbm, b1_v, sem_small.at[1])

    def b2_copy():
        return pltpu.make_async_copy(b2_hbm, b2_v, sem_small.at[2])

    def wq_copy():
        return pltpu.make_async_copy(wq_hbm, wq_v, sem_w.at[0])

    def w1_copy():
        return pltpu.make_async_copy(w1_hbm, w1_v, sem_w.at[1])

    def w2_copy():
        return pltpu.make_async_copy(w2t_hbm, w2t_v, sem_w.at[2])

    def k_copy(h):
        return pltpu.make_async_copy(
            k_hbm.at[:, h, pl.ds(seq - window, window), :], kbuf.at[h], sem_k.at[h])

    def v_copy(h):
        return pltpu.make_async_copy(
            v_hbm.at[:, h, pl.ds(seq - window, window), :], vbuf.at[h], sem_v.at[h])

    def wo_copy(c):
        r0, nr, c0, nc = wo_pieces[c]
        idx = (pl.ds(r0, nr), pl.ds(c0, nc))
        return pltpu.make_async_copy(wot_hbm.at[idx], wot_v.at[idx], sem_wo.at[c])

    wq_copy().start()
    x_copy().start()
    b1_copy().start()
    b2_copy().start()
    w1_copy().start()
    w2_copy().start()

    def issue(h, carry):
        k_copy(h).start()
        v_copy(h).start()
        return carry

    lax.fori_loop(0, n_kv, issue, 0)
    for c in range(len(wo_pieces)):
        wo_copy(c).start()

    x_copy().wait()
    x = x_v[...].astype(jnp.float32)
    x8 = jnp.concatenate([x] * (_ROWS // n_batch), axis=0)
    mu = jnp.mean(x8, axis=-1, keepdims=True)
    xc = x8 - mu
    var = jnp.mean(xc * xc, axis=-1, keepdims=True)
    xn8 = (xc / jnp.sqrt(var + _EPS)).astype(jnp.bfloat16)

    wq_copy().wait()
    q_scr[...] = jnp.dot(xn8, wq_v[...], preferred_element_type=jnp.float32)

    b1_copy().wait()
    b2_copy().wait()
    w1_copy().wait()
    hid = jnp.dot(xn8, w1_v[...], preferred_element_type=jnp.float32)
    hid = hid + b1_v[...].astype(jnp.float32).reshape(1, -1)
    hid = jax.nn.gelu(hid, approximate=True).astype(jnp.bfloat16)
    w2_copy().wait()
    y = lax.dot_general(hid, w2t_v[...], _NT, preferred_element_type=jnp.float32)
    y = y + b2_v[...].astype(jnp.float32).reshape(1, -1)
    gate = y * jax.nn.sigmoid(y)

    scale = _DH ** -0.5
    row = lax.broadcasted_iota(jnp.int32, (_ROWS, _DH), 0)
    srow = lax.broadcasted_iota(jnp.int32, (_ROWS, window), 0)

    def attend(h, carry):
        c0 = pl.multiple_of(h * (rep * _DH), rep * _DH)
        c1 = pl.multiple_of(h * (rep * _DH) + _DH, _DH)
        qh = jnp.where((row & 2) == 0, q_scr[:, pl.ds(c0, _DH)], q_scr[:, pl.ds(c1, _DH)])
        qh = qh.astype(jnp.bfloat16)
        k_copy(h).wait()
        s0 = lax.dot_general(qh, kbuf[h, 0], _NT, preferred_element_type=jnp.float32)
        s1 = lax.dot_general(qh, kbuf[h, 1], _NT, preferred_element_type=jnp.float32)
        s = jnp.where((srow & 1) == 0, s0, s1) * scale
        m = jnp.max(s, axis=-1, keepdims=True)
        p = jnp.exp(s - m)
        l = jnp.sum(p, axis=-1, keepdims=True)
        pb = p.astype(jnp.bfloat16)
        v_copy(h).wait()
        o0 = jnp.dot(pb, vbuf[h, 0], preferred_element_type=jnp.float32)
        o1 = jnp.dot(pb, vbuf[h, 1], preferred_element_type=jnp.float32)
        o = jnp.where((row & 1) == 0, o0, o1) / l
        o_scr[:, pl.ds(c0, _DH)] = o
        o_scr[:, pl.ds(c1, _DH)] = pltpu.roll(o, _ROWS - 2, 0)
        return carry

    lax.fori_loop(0, n_kv, attend, 0)

    partial = {}
    for c, (r0, nr, c0, nc) in enumerate(wo_pieces):
        oc = o_scr[:, c0:c0 + nc].astype(jnp.bfloat16)
        closes_group = c0 + nc == _HQ * _DH
        if closes_group:
            gs = gate[:, r0:r0 + nr]
            base = x8[:, r0:r0 + nr]
            if r0 in partial:
                base = base + partial[r0] * gs
        wo_copy(c).wait()
        part = lax.dot_general(oc, wot_v[r0:r0 + nr, c0:c0 + nc], _NT,
                               preferred_element_type=jnp.float32)
        if closes_group:
            res = base + part * gs
            out_ref[:, r0:r0 + nr] = res[0:n_batch].astype(out_ref.dtype)
        else:
            partial[r0] = part if r0 not in partial else partial[r0] + part


def _wo_pieces(d_model, k_total):
    pieces = []
    r = 0
    while d_model - r >= 128:
        pieces.append((r, 128, 0, k_total))
        r += 128
    if r < d_model:
        head = (k_total * 5 // 8) // 128 * 128
        pieces.append((r, d_model - r, 0, head))
        pieces.append((r, d_model - r, head, k_total - head))
    return tuple(pieces)


@jax.jit
def pallas_recurrent_scan__sliding_block_cached__dense_activation_gelu__decode_kernel(
    A_x: jax.Array,
    A_k_cache: jax.Array,
    A_v_cache: jax.Array,
    A_wq: jax.Array,
    A_wo: jax.Array,
    B_x: jax.Array,
    B_w1: jax.Array,
    B_b1: jax.Array,
    B_w2: jax.Array,
    B_b2: jax.Array,
):
    del B_x
    n_batch, sq, d_model = A_x.shape
    _, n_kv, seq, dh = A_k_cache.shape
    assert sq == 1 and dh == _DH
    window = min(4096, max(256, seq // 4))
    d_ff = B_w1.shape[1]
    wo_pieces = _wo_pieces(d_model, _HQ * _DH)
    bf16 = jnp.bfloat16

    hbm = pl.BlockSpec(memory_space=pl.ANY)
    out = pl.pallas_call(
        functools.partial(_kernel, n_batch=n_batch, n_kv=n_kv, window=window, seq=seq,
                          wo_pieces=wo_pieces),
        out_shape=jax.ShapeDtypeStruct((n_batch, d_model), A_x.dtype),
        in_specs=[hbm] * 9,
        out_specs=pl.BlockSpec(memory_space=pltpu.VMEM),
        scratch_shapes=[
            pltpu.VMEM((n_batch, d_model), bf16),
            pltpu.VMEM((d_ff,), bf16),
            pltpu.VMEM((d_model,), bf16),
            pltpu.VMEM((d_model, _HQ * _DH), bf16),
            pltpu.VMEM((d_model, d_ff), bf16),
            pltpu.VMEM((d_model, d_ff), bf16),
            pltpu.VMEM((d_model, _HQ * _DH), bf16),
            pltpu.VMEM((n_kv, n_batch, window, _DH), bf16),
            pltpu.VMEM((n_kv, n_batch, window, _DH), bf16),
            pltpu.VMEM((_ROWS, _HQ * _DH), jnp.float32),
            pltpu.VMEM((_ROWS, _HQ * _DH), jnp.float32),
            pltpu.SemaphoreType.DMA((3,)),
            pltpu.SemaphoreType.DMA((3,)),
            pltpu.SemaphoreType.DMA((n_kv,)),
            pltpu.SemaphoreType.DMA((n_kv,)),
            pltpu.SemaphoreType.DMA((len(wo_pieces),)),
        ],
        compiler_params=pltpu.CompilerParams(
            vmem_limit_bytes=112 * 1024 * 1024,
            disable_semaphore_checks=True,
        ),
    )(A_x.reshape(n_batch, d_model), A_k_cache, A_v_cache, A_wq, A_wo.T,
      B_w1, B_b1, B_w2.T, B_b2)
    return out.reshape(n_batch, sq, d_model)
```

```python
import functools

import jax
import jax.numpy as jnp
from jax import lax
import jax.experimental.pallas as pl
import jax.experimental.pallas.tpu as pltpu

_NT = (((1,), (1,)), ((), ()))
_HQ = 32
_DH = 128
_ROWS = 8
_EPS = 1e-5
_SIDE_ROWS = 432
_SIDE_EXTRA = 2
_SIDE_LEAD = 4
_LOOKAHEAD = 2


def _kernel(x_hbm, k_hbm, v_hbm, wq_hbm, wot_hbm, w1_hbm, b1_hbm, w2t_hbm, b2_hbm,
            out_ref,
            x_v, b1_v, b2_v, wq_v, w1_v, w2t_v, wot_v, kbuf, vbuf, q_scr, o_scr, stage,
            sem_small, sem_w, sem_k, sem_v, sem_vt, sem_wo, sem_in, sem_out,
            *, n_batch, n_kv, window, seq, wo_pieces):
    rep = _HQ // n_kv
    assert rep == 2 and n_batch == 2
    w0 = seq - window
    body = window - _SIDE_ROWS
    n_side = n_kv + _SIDE_EXTRA
    n_vt = n_kv - _SIDE_EXTRA
    assert _SIDE_LEAD - 2 == _SIDE_EXTRA and n_side + 1 == n_kv - 1 + _SIDE_LEAD

    def x_copy():
        return pltpu.make_async_copy(x_hbm, x_v, sem_small.at[0])

    def b1_copy():
        return pltpu.make_async_copy(b1_hbm, b1_v, sem_small.at[1])

    def b2_copy():
        return pltpu.make_async_copy(b2_hbm, b2_v, sem_small.at[2])

    def wq_copy():
        return pltpu.make_async_copy(wq_hbm, wq_v, sem_w.at[0])

    def w1_copy():
        return pltpu.make_async_copy(w1_hbm, w1_v, sem_w.at[1])

    def w2_copy():
        return pltpu.make_async_copy(w2t_hbm, w2t_v, sem_w.at[2])

    def k_copy(h):
        return pltpu.make_async_copy(
            k_hbm.at[:, h, pl.ds(w0, window), :], kbuf.at[h], sem_k.at[h])

    def v_copy(h):
        return pltpu.make_async_copy(
            v_hbm.at[:, h, pl.ds(w0, body), :], vbuf.at[h, :, pl.ds(0, body), :], sem_v.at[h])

    def vt_copy(h):
        return pltpu.make_async_copy(
            v_hbm.at[0, h, pl.ds(w0 + body, _SIDE_ROWS), :],
            vbuf.at[h, 0, pl.ds(body, _SIDE_ROWS), :], sem_vt.at[h])

    def wo_copy(c):
        r0, nr, c0, nc = wo_pieces[c]
        idx = (pl.ds(r0, nr), pl.ds(c0, nc))
        return pltpu.make_async_copy(wot_hbm.at[idx], wot_v.at[idx], sem_wo.at[c])

    def when(cond):
        if isinstance(cond, bool):
            return (lambda f: f()) if cond else (lambda f: None)
        return pl.when(cond)

    def issue_head(h):
        k_copy(h).start()
        v_copy(h).start()

        @when(h < n_vt)
        def _():
            vt_copy(h).start()

    def side_bh(j):
        if isinstance(j, int):
            return (0, n_vt + j) if j < _SIDE_EXTRA else (1, j - _SIDE_EXTRA)
        early = j < _SIDE_EXTRA
        return jnp.where(early, 0, 1), jnp.where(early, n_vt + j, j - _SIDE_EXTRA)

    def side_in(j):
        b, h = side_bh(j)
        return pltpu.make_async_copy(
            v_hbm.at[b, h, pl.ds(w0 + body, _SIDE_ROWS), :], stage.at[j % 2], sem_in.at[j % 2])

    def side_out(j):
        b, h = side_bh(j)
        return pltpu.make_async_copy(
            stage.at[j % 2], vbuf.at[h, b, pl.ds(body, _SIDE_ROWS), :], sem_out.at[j % 2])

    def side_step(j):
        @when((j >= 1) & (j - 1 < n_side))
        def _():
            side_in(j - 1).wait()
            side_out(j - 1).start()

        @when((j >= 2) & (j - 2 < n_side))
        def _():
            side_out(j - 2).wait()

        @when(j < n_side)
        def _():
            side_in(j).start()

    wq_copy().start()
    side_step(0)
    x_copy().start()
    b1_copy().start()
    b2_copy().start()
    w1_copy().start()
    w2_copy().start()
    for h in range(_LOOKAHEAD):
        issue_head(h)

    x_copy().wait()
    x = x_v[...].astype(jnp.float32)
    x8 = jnp.concatenate([x] * (_ROWS // n_batch), axis=0)
    mu = jnp.mean(x8, axis=-1, keepdims=True)
    xc = x8 - mu
    var = jnp.mean(xc * xc, axis=-1, keepdims=True)
    xn8 = (xc / jnp.sqrt(var + _EPS)).astype(jnp.bfloat16)

    wq_copy().wait()
    side_step(1)
    q_scr[...] = jnp.dot(xn8, wq_v[...], preferred_element_type=jnp.float32)

    b1_copy().wait()
    b2_copy().wait()
    w1_copy().wait()
    side_step(2)
    hid = jnp.dot(xn8, w1_v[...], preferred_element_type=jnp.float32)
    hid = hid + b1_v[...].astype(jnp.float32).reshape(1, -1)
    hid = jax.nn.gelu(hid, approximate=True).astype(jnp.bfloat16)
    w2_copy().wait()
    side_step(3)
    y = lax.dot_general(hid, w2t_v[...], _NT, preferred_element_type=jnp.float32)
    y = y + b2_v[...].astype(jnp.float32).reshape(1, -1)
    gate = y * jax.nn.sigmoid(y)

    scale = _DH ** -0.5
    row = lax.broadcasted_iota(jnp.int32, (_ROWS, _DH), 0)
    srow = lax.broadcasted_iota(jnp.int32, (_ROWS, window), 0)

    def attend(h, carry):
        @pl.when(h + _LOOKAHEAD < n_kv)
        def _():
            issue_head(h + _LOOKAHEAD)

        @pl.when(h + _LOOKAHEAD == n_kv)
        def _():
            for c in range(len(wo_pieces)):
                wo_copy(c).start()

        c0 = pl.multiple_of(h * (rep * _DH), rep * _DH)
        c1 = pl.multiple_of(h * (rep * _DH) + _DH, _DH)
        qh = jnp.where((row & 2) == 0, q_scr[:, pl.ds(c0, _DH)], q_scr[:, pl.ds(c1, _DH)])
        qh = qh.astype(jnp.bfloat16)
        k_copy(h).wait()
        s0 = lax.dot_general(qh, kbuf[h, 0], _NT, preferred_element_type=jnp.float32)
        s1 = lax.dot_general(qh, kbuf[h, 1], _NT, preferred_element_type=jnp.float32)
        s = jnp.where((srow & 1) == 0, s0, s1) * scale
        m = jnp.max(s, axis=-1, keepdims=True)
        p = jnp.exp(s - m)
        l = jnp.sum(p, axis=-1, keepdims=True)
        pb = p.astype(jnp.bfloat16)
        v_copy(h).wait()

        @pl.when(h < n_vt)
        def _():
            vt_copy(h).wait()

        side_step(h + _SIDE_LEAD)
        o0 = jnp.dot(pb, vbuf[h, 0], preferred_element_type=jnp.float32)
        o1 = jnp.dot(pb, vbuf[h, 1], preferred_element_type=jnp.float32)
        o = jnp.where((row & 1) == 0, o0, o1) / l
        o_scr[:, pl.ds(c0, _DH)] = o
        o_scr[:, pl.ds(c1, _DH)] = pltpu.roll(o, _ROWS - 2, 0)
        return carry

    lax.fori_loop(0, n_kv, attend, 0)

    partial = {}
    for c, (r0, nr, c0, nc) in enumerate(wo_pieces):
        oc = o_scr[:, c0:c0 + nc].astype(jnp.bfloat16)
        closes_group = c0 + nc == _HQ * _DH
        if closes_group:
            gs = gate[:, r0:r0 + nr]
            base = x8[:, r0:r0 + nr]
            if r0 in partial:
                base = base + partial[r0] * gs
        wo_copy(c).wait()
        part = lax.dot_general(oc, wot_v[r0:r0 + nr, c0:c0 + nc], _NT,
                               preferred_element_type=jnp.float32)
        if closes_group:
            res = base + part * gs
            out_ref[:, r0:r0 + nr] = res[0:n_batch].astype(out_ref.dtype)
        else:
            partial[r0] = part if r0 not in partial else partial[r0] + part


def _wo_pieces(d_model, k_total):
    pieces = []
    r = 0
    while d_model - r >= 128:
        pieces.append((r, 128, 0, k_total))
        r += 128
    if r < d_model:
        head = (k_total * 5 // 8) // 128 * 128
        pieces.append((r, d_model - r, 0, head))
        pieces.append((r, d_model - r, head, k_total - head))
    return tuple(pieces)


@jax.jit
def pallas_recurrent_scan__sliding_block_cached__dense_activation_gelu__decode_kernel(
    A_x: jax.Array,
    A_k_cache: jax.Array,
    A_v_cache: jax.Array,
    A_wq: jax.Array,
    A_wo: jax.Array,
    B_x: jax.Array,
    B_w1: jax.Array,
    B_b1: jax.Array,
    B_w2: jax.Array,
    B_b2: jax.Array,
):
    del B_x
    n_batch, sq, d_model = A_x.shape
    _, n_kv, seq, dh = A_k_cache.shape
    assert sq == 1 and dh == _DH
    window = min(4096, max(256, seq // 4))
    assert window > _SIDE_ROWS
    d_ff = B_w1.shape[1]
    wo_pieces = _wo_pieces(d_model, _HQ * _DH)
    bf16 = jnp.bfloat16

    hbm = pl.BlockSpec(memory_space=pl.ANY)
    out = pl.pallas_call(
        functools.partial(_kernel, n_batch=n_batch, n_kv=n_kv, window=window, seq=seq,
                          wo_pieces=wo_pieces),
        out_shape=jax.ShapeDtypeStruct((n_batch, d_model), A_x.dtype),
        in_specs=[hbm] * 9,
        out_specs=pl.BlockSpec(memory_space=pltpu.VMEM),
        scratch_shapes=[
            pltpu.VMEM((n_batch, d_model), bf16),
            pltpu.VMEM((d_ff,), bf16),
            pltpu.VMEM((d_model,), bf16),
            pltpu.VMEM((d_model, _HQ * _DH), bf16),
            pltpu.VMEM((d_model, d_ff), bf16),
            pltpu.VMEM((d_model, d_ff), bf16),
            pltpu.VMEM((d_model, _HQ * _DH), bf16),
            pltpu.VMEM((n_kv, n_batch, window, _DH), bf16),
            pltpu.VMEM((n_kv, n_batch, window, _DH), bf16),
            pltpu.VMEM((_ROWS, _HQ * _DH), jnp.float32),
            pltpu.VMEM((_ROWS, _HQ * _DH), jnp.float32),
            pltpu.SMEM((2, _SIDE_ROWS, _DH), bf16),
            pltpu.SemaphoreType.DMA((3,)),
            pltpu.SemaphoreType.DMA((3,)),
            pltpu.SemaphoreType.DMA((n_kv,)),
            pltpu.SemaphoreType.DMA((n_kv,)),
            pltpu.SemaphoreType.DMA((n_kv,)),
            pltpu.SemaphoreType.DMA((len(wo_pieces),)),
            pltpu.SemaphoreType.DMA((2,)),
            pltpu.SemaphoreType.DMA((2,)),
        ],
        compiler_params=pltpu.CompilerParams(
            vmem_limit_bytes=112 * 1024 * 1024,
            disable_semaphore_checks=True,
        ),
    )(A_x.reshape(n_batch, d_model), A_k_cache, A_v_cache, A_wq, A_wo.T,
      B_w1, B_b1, B_w2.T, B_b2)
    return out.reshape(n_batch, sq, d_model)
```
